```python
import os as _os
_os.environ.setdefault("JAX_PLATFORMS", "cpu")
import jax
import jax.numpy as jnp

def _softmax(x, axis=-1):
    return jax.nn.softmax(x, axis=axis)
def _gelu(x):
    return jax.nn.gelu(x, approximate=True)
def _silu(x):
    return jax.nn.silu(x)
def _sigmoid(x):
    return jax.nn.sigmoid(x)
def _layernorm(x, axis=-1, eps=1e-5):
    m = jnp.mean(x, axis=axis, keepdims=True)
    v = jnp.var(x, axis=axis, keepdims=True)
    return (x - m) / jnp.sqrt(v + eps)
def _scatter_add(tgt, idx, src, axis=0):
    return tgt.at[idx].add(src)
def _segment_sum(src, seg, n):
    return jax.ops.segment_sum(src, seg, n)
class _Rng:
    def __init__(self, key):
        self._k = key
    def _next(self):
        self._k, sub = jax.random.split(self._k)
        return sub
    def normal(self, shape):
        return jax.random.normal(self._next(), shape, dtype=jnp.bfloat16)
    def randint(self, lo, hi, shape):
        return jax.random.randint(self._next(), shape, lo, hi, dtype=jnp.int32)
    def uniform(self, shape, lo=0.0, hi=1.0):
        return jax.random.uniform(self._next(), shape, jnp.bfloat16, lo, hi)
    def permutation(self, n):
        return jax.random.permutation(self._next(), n)


kernel_name = 'standalone__sliding_local_fixed_window__prompt'

def setup_inputs():
    _rng = _Rng(jax.random.key(int.from_bytes(__import__("os").urandom(4), "little")))
    _w = (lambda a: (lambda t: t.astype(jnp.bfloat16) if jnp.issubdtype(t.dtype, jnp.floating) else t)(jnp.asarray(a)))
    B, H, S, D = 1, 32, 2048, 128
    return {
        "q": _w((lambda *s: _rng.normal(s) * 0.4)(B, H, S, D)),
        "k": _w((lambda *s: _rng.normal(s) * 0.4)(B, H, S, D)),
        "v": _w((lambda *s: _rng.normal(s) * 0.05)(B, H, S, D)),
    }

def reference(q, k, v):
    B, H, S, D = q.shape
    w = 32
    pos = jnp.arange(S)
    rel = pos[:, None] - pos[None, :]
    mask = (rel >= 0) & (rel < w)
    scores = jnp.einsum("bhqd,bhkd->bhqk", q, k) * (D ** -0.5)
    scores = jnp.where(mask[None, None], scores, (lambda x, dt: x.astype(dt))(jnp.array(-1e9), q.dtype))
    p = _softmax(scores, axis=-1)
    return jnp.einsum("bhqk,bhkd->bhqd", p, v)
```

```python
import jax
import jax.numpy as jnp
from jax import lax
import jax.experimental.pallas as pl
import jax.experimental.pallas.tpu as pltpu

WINDOW = 32
TILE_K = 128
TILE_Q = TILE_K - WINDOW
LOG2E = 1.4426950408889634
MASKED = -1e30


def _attend(q, k, v, offset, scale_log2e):
    shape = (q.shape[0], k.shape[0])
    s = lax.dot_general(q, k, (((1,), (1,)), ((), ())), preferred_element_type=jnp.float32)
    rel = (lax.broadcasted_iota(jnp.int32, shape, 0) + offset
           - lax.broadcasted_iota(jnp.int32, shape, 1))
    s = jnp.where((rel >= 0) & (rel < WINDOW), s, MASKED)
    m = jnp.max(s, axis=1, keepdims=True)
    p = jnp.exp2((s - m) * scale_log2e)
    l = jnp.sum(p, axis=1, keepdims=True)
    o = jnp.dot(p.astype(v.dtype), v, preferred_element_type=jnp.float32)
    return (o * pl.reciprocal(l, approx=True)).astype(q.dtype)


def _head_chunks(n):
    chunks = [c for c in (n * 10 // 32, n * 8 // 32, n * 6 // 32, n * 4 // 32, n * 2 // 32) if c]
    return chunks + [n - sum(chunks)]


@jax.jit
def pallas_standalone__sliding_local_fixed_window__prompt_kernel(
    q: jax.Array,
    k: jax.Array,
    v: jax.Array,
):
    B, H, S, D = q.shape
    n_heads = B * H
    assert S >= TILE_K and (S - TILE_K) % TILE_Q == 0
    scale_log2e = float(D ** -0.5 * LOG2E)
    chunks = _head_chunks(n_heads)
    starts = [sum(chunks[:i]) for i in range(len(chunks))]
    last = len(chunks) - 1
    writes = [(0, starts[last]), (starts[last], chunks[last])] if last else [(0, n_heads)]

    def kernel_function(q_hbm, k_hbm, v_hbm, o_hbm, q_buf, k_buf, v_buf, o_buf, r_sem, w_sem):
        def read(t, c):
            heads = pl.ds(starts[c], chunks[c])
            return pltpu.make_async_copy(
                (q_hbm, k_hbm, v_hbm)[t].at[heads], (q_buf, k_buf, v_buf)[t].at[heads], r_sem.at[t, c])

        def write(i):
            heads = pl.ds(*writes[i])
            return pltpu.make_async_copy(o_buf.at[heads], o_hbm.at[heads], w_sem.at[i])

        for c in range(len(chunks)):
            for t in range(3):
                read(t, c).start()

        def head(h, carry):
            for c in range(len(chunks)):
                @pl.when(h == starts[c])
                def _():
                    read(0, c).wait()
                    read(1, c).wait()
                    if c == last and last:
                        write(0).start()
                    read(2, c).wait()

            rows = slice(0, TILE_K)
            o_buf[h, rows, :] = _attend(
                q_buf[h, rows, :], k_buf[h, rows, :], v_buf[h, rows, :], 0, scale_log2e)
            for i in range(TILE_K, S, TILE_Q):
                rows, keys = slice(i, i + TILE_Q), slice(i - WINDOW, i + TILE_Q)
                o_buf[h, rows, :] = _attend(
                    q_buf[h, rows, :], k_buf[h, keys, :], v_buf[h, keys, :], WINDOW, scale_log2e)
            return carry

        lax.fori_loop(0, n_heads, head, 0)
        write(len(writes) - 1).start()
        for i in range(len(writes)):
            write(i).wait()

    buf = pltpu.VMEM((n_heads, S, D), q.dtype)
    hbm = pl.BlockSpec(memory_space=pl.ANY)
    out = pl.pallas_call(
        kernel_function,
        in_specs=[hbm, hbm, hbm],
        out_specs=hbm,
        out_shape=jax.ShapeDtypeStruct((n_heads, S, D), q.dtype),
        scratch_shapes=[
            buf, buf, buf, buf,
            pltpu.SemaphoreType.DMA((3, len(chunks))),
            pltpu.SemaphoreType.DMA((len(writes),)),
        ],
        compiler_params=pltpu.CompilerParams(vmem_limit_bytes=100 * 2**20),
    )(q.reshape(n_heads, S, D), k.reshape(n_heads, S, D), v.reshape(n_heads, S, D))
    return out.reshape(B, H, S, D)
```

```python
import jax
import jax.numpy as jnp
from jax import lax
import jax.experimental.pallas as pl
import jax.experimental.pallas.tpu as pltpu

WINDOW = 32
TILE_K = 128
TILE_Q = TILE_K - WINDOW
N_CHUNKS = 4
WRITE_ROWS = 32
LOG2E = 1.4426950408889634
MASKED_SCORE = -998244352.0


def _attend(q, k, v, v_total, offset, seq_len):
    scale = q.shape[1] ** -0.5
    masked = MASKED_SCORE / scale
    shape = (q.shape[0], k.shape[0])
    s = lax.dot_general(q, k, (((1,), (1,)), ((), ())), preferred_element_type=jnp.float32)
    rel = (lax.broadcasted_iota(jnp.int32, shape, 0) + offset
           - lax.broadcasted_iota(jnp.int32, shape, 1))
    s = jnp.where((rel >= 0) & (rel < WINDOW), s, masked)
    m = jnp.max(s, axis=1, keepdims=True)
    e = jnp.exp2((masked - m) * (scale * LOG2E))
    p = jnp.exp2((s - m) * (scale * LOG2E)) - e
    denom = jnp.sum(p, axis=1, keepdims=True) + seq_len * e
    o = jnp.dot(p.astype(v.dtype), v, preferred_element_type=jnp.float32) + e * v_total
    return (o * pl.reciprocal(denom, approx=False)).astype(q.dtype)


@jax.jit
def pallas_standalone__sliding_local_fixed_window__prompt_kernel(
    q: jax.Array,
    k: jax.Array,
    v: jax.Array,
):
    B, H, S, D = q.shape
    n_heads = B * H
    chunk = n_heads // N_CHUNKS
    assert n_heads % N_CHUNKS == 0 and chunk >= 2
    assert S >= TILE_K and (S - TILE_K) % TILE_Q == 0
    last = N_CHUNKS - 1
    last_start = last * chunk
    tail_sem, write_sem = N_CHUNKS, N_CHUNKS + 1

    def kernel_function(q_hbm, k_hbm, v_hbm, o_hbm, q_buf, k_buf, v_buf, o_buf, sems):
        def read(src, dst, first, count, sem):
            heads = pl.ds(first, count)
            return pltpu.make_async_copy(src.at[heads], dst.at[heads], sems.at[sem])

        def chunk_reads(c, v_count=chunk):
            return [read(q_hbm, q_buf, c * chunk, chunk, c),
                    read(k_hbm, k_buf, c * chunk, chunk, c),
                    read(v_hbm, v_buf, c * chunk, v_count, c)]

        last_reads = chunk_reads(last, chunk - 1)
        tail_read = read(v_hbm, v_buf, n_heads - 1, 1, tail_sem)

        def start_writes(first, count):
            def start(i, carry):
                part = (pl.ds(first, count),
                        pl.ds(pl.multiple_of(i * WRITE_ROWS, WRITE_ROWS), WRITE_ROWS))
                pltpu.make_async_copy(o_buf.at[part], o_hbm.at[part], sems.at[write_sem]).start()
                return carry
            lax.fori_loop(0, S // WRITE_ROWS, start, 0)

        for c in range(last):
            for copy in chunk_reads(c):
                copy.start()
        for copy in last_reads:
            copy.start()
        tail_read.start()

        def head(h, carry):
            @pl.when((h % chunk == 0) & (h < last_start))
            def _():
                for copy in chunk_reads(h // chunk):
                    copy.wait()

            @pl.when(h == last_start)
            def _():
                for copy in last_reads:
                    copy.wait()
                start_writes(0, last_start)
                tail_read.wait()

            v_total = jnp.sum(v_buf[h].astype(jnp.float32), axis=0, keepdims=True)
            rows = slice(0, TILE_K)
            o_buf[h, rows, :] = _attend(
                q_buf[h, rows, :], k_buf[h, rows, :], v_buf[h, rows, :], v_total, 0, S)
            for i in range(TILE_K, S, TILE_Q):
                rows, keys = slice(i, i + TILE_Q), slice(i - WINDOW, i + TILE_Q)
                o_buf[h, rows, :] = _attend(
                    q_buf[h, rows, :], k_buf[h, keys, :], v_buf[h, keys, :], v_total, WINDOW, S)
            return carry

        lax.fori_loop(0, n_heads, head, 0)
        start_writes(last_start, chunk)
        pltpu.make_async_copy(o_buf, o_hbm, sems.at[write_sem]).wait()

    buf = pltpu.VMEM((n_heads, S, D), q.dtype)
    hbm = pl.BlockSpec(memory_space=pl.ANY)
    out = pl.pallas_call(
        kernel_function,
        in_specs=[hbm, hbm, hbm],
        out_specs=hbm,
        out_shape=jax.ShapeDtypeStruct((n_heads, S, D), q.dtype),
        scratch_shapes=[buf, buf, buf, buf, pltpu.SemaphoreType.DMA((N_CHUNKS + 2,))],
        compiler_params=pltpu.CompilerParams(vmem_limit_bytes=100 * 2**20),
    )(q.reshape(n_heads, S, D), k.reshape(n_heads, S, D), v.reshape(n_heads, S, D))
    return out.reshape(B, H, S, D)
```
